```python
import os as _os
_os.environ.setdefault("JAX_PLATFORMS", "cpu")
import jax
import jax.numpy as jnp

def _softmax(x, axis=-1):
    return jax.nn.softmax(x, axis=axis)
def _gelu(x):
    return jax.nn.gelu(x, approximate=True)
def _silu(x):
    return jax.nn.silu(x)
def _sigmoid(x):
    return jax.nn.sigmoid(x)
def _layernorm(x, axis=-1, eps=1e-5):
    m = jnp.mean(x, axis=axis, keepdims=True)
    v = jnp.var(x, axis=axis, keepdims=True)
    return (x - m) / jnp.sqrt(v + eps)
def _scatter_add(tgt, idx, src, axis=0):
    return tgt.at[idx].add(src)
def _segment_sum(src, seg, n):
    return jax.ops.segment_sum(src, seg, n)
class _Rng:
    def __init__(self, key):
        self._k = key
    def _next(self):
        self._k, sub = jax.random.split(self._k)
        return sub
    def normal(self, shape):
        return jax.random.normal(self._next(), shape, dtype=jnp.bfloat16)
    def randint(self, lo, hi, shape):
        return jax.random.randint(self._next(), shape, lo, hi, dtype=jnp.int32)
    def uniform(self, shape, lo=0.0, hi=1.0):
        return jax.random.uniform(self._next(), shape, jnp.bfloat16, lo, hi)
    def permutation(self, n):
        return jax.random.permutation(self._next(), n)


kernel_name = 'sequential_preLN__softmax_full_mha__swiglu_ffn__prompt'

def setup_inputs():
    _rng = _Rng(jax.random.key(int.from_bytes(__import__("os").urandom(4), "little")))
    _w = (lambda a: (lambda t: t.astype(jnp.bfloat16) if jnp.issubdtype(t.dtype, jnp.floating) else t)(jnp.asarray(a)))
    def _A_setup():
        B, S, D = 1, 2048, 512
        return {
            "x": _w((lambda *s: _rng.normal(s) * 0.05)(B, S, D)),
            "wqkv": _w((lambda *s: _rng.normal(s) * 0.05)(D, 3 * D)),
            "wo": _w((lambda *s: _rng.normal(s) * 0.05)(D, D)),
        }
    _A_in = _A_setup()

    def _B_setup():
        B, S, D, F = 1, 2048, 512, 1792
        return {
            "x": _w((lambda *s: _rng.normal(s) * 0.05)(B, S, D)),
            "w_gate": _w((lambda *s: _rng.normal(s) * 0.05)(D, F)),
            "w_up": _w((lambda *s: _rng.normal(s) * 0.05)(D, F)),
            "w_down": _w((lambda *s: _rng.normal(s) * 0.05)(F, D)),
        }
    _B_in = _B_setup()

    return {
        "A_x": _A_in["x"],
        "A_wqkv": _A_in["wqkv"],
        "A_wo": _A_in["wo"],
        "B_x": _B_in["x"],
        "B_w_gate": _B_in["w_gate"],
        "B_w_up": _B_in["w_up"],
        "B_w_down": _B_in["w_down"],
    }

def reference(A_x, A_wqkv, A_wo, B_x, B_w_gate, B_w_up, B_w_down):
    def _A_ref(x, wqkv, wo):
        B, S, D = x.shape
        H = 32; Dh = D // H
        qkv = (lambda x, *d: x.transpose(*d))((x @ wqkv).reshape(B, S, 3, H, Dh), 2, 0, 3, 1, 4)
        q, k, v = qkv[0], qkv[1], qkv[2]
        scale = Dh ** -0.5
        scores = jnp.einsum("bhqd,bhkd->bhqk", q, k) * scale
        p = _softmax(scores, axis=-1)
        o = jnp.einsum("bhqk,bhkd->bhqd", p, v)
        return (lambda x, *d: x.transpose(*d))(o, 0, 2, 1, 3).reshape(B, S, D) @ wo

    def _B_ref(x, w_gate, w_up, w_down):
        g = _silu(x @ w_gate)
        u = x @ w_up
        return (g * u) @ w_down

    x = A_x
    h = x + _A_ref(_layernorm(x, axis=-1), A_wqkv, A_wo)
    h2 = h + _B_ref(_layernorm(h, axis=-1), B_w_gate, B_w_up, B_w_down)
    return h2
```

```python
import functools
import math

import jax
import jax.numpy as jnp
from jax import lax
import jax.experimental.pallas as pl
import jax.experimental.pallas.tpu as pltpu

_H = 32
_EPS = 1e-5
_QB = 512
_KC = 128
_RB = 256
_PK = 16
_CK = (1, 3, 5, 7, 9, 11, 13)
_PQ = 256
_DS = 8
_C1 = 15
_TK = 3
_FJ = 6

_F32 = jnp.float32
_BF16 = jnp.bfloat16
_TN = (((0,), (0,)), ((), ()))


def _layernorm(x):
    m = jnp.mean(x, axis=-1, keepdims=True)
    c = x - m
    v = jnp.mean(c * c, axis=-1, keepdims=True)
    return c * lax.rsqrt(v + _EPS)


def _aligned(start, size):
    return pl.ds(start if isinstance(start, int) else pl.multiple_of(start, size), size)


def _add(total, x):
    return x if total is None else total + x


def _pack(x):
    return pltpu.bitcast(x.astype(_BF16), jnp.uint32)


def _unpack(x):
    return pltpu.bitcast(x, _BF16)


def _lhs7(a11, a12, a21, a22):
    return (a11 + a22, a21 + a22, a11, a22, a11 + a12, a21 - a11, a12 - a22)


def _rhs5(b11, b12, b21, b22):
    return (b11 + b22, b12 - b22, b21 - b11, b11 + b12, b21 + b22)


def _rhs7(sums, b11, b22):
    return (sums[0], b11, sums[1], sums[2], b22, sums[3], sums[4])


def _out4(m):
    return ((m[0] + m[3]) + (m[6] - m[4]), m[2] + m[4],
            m[1] + m[3], (m[0] - m[1]) + (m[2] + m[5]))


def _block_kernel(x_hbm, wqkv_hbm, wo_hbm, wg_hbm, wu_hbm, wd_hbm, out_hbm,
                  x_v, wqkv_v, wo_v, wgu_v, wd_v,
                  k_v, qt_v, vt_v, ot_v, s_v, qb_v, kb_v,
                  xn_v, hp_v, h_v, hx_v, hn_v, a_v, w5_v, d5_v, out_v,
                  spare_s, x_sem, q_sem, w_sem, o_sem, *, S, D, F):
    DH = D // _H
    NQ = S // _QB
    NC = S // _KC
    HPG = 128 // DH
    qscale = (DH ** -0.5) * math.log2(math.e)

    def x_copy(r):
        rows = pl.ds(r * _QB, _QB)
        return pltpu.make_async_copy(x_hbm.at[rows], x_v.at[rows], x_sem.at[r])

    def out_copy(r):
        return pltpu.make_async_copy(
            out_v.at[r], out_hbm.at[pl.ds(r * _RB, _RB)], o_sem.at[r])

    w_copies = [
        pltpu.make_async_copy(src, dst, w_sem.at[i])
        for i, (src, dst) in enumerate(
            ((wg_hbm, wgu_v.at[0, 0:D]), (wu_hbm, wgu_v.at[1, 0:D]),
             (wd_hbm, wd_v.at[0:F]), (wo_hbm, wo_v)))
    ]

    def block_rows(r):
        return _aligned(r * _QB, _QB)

    def norm_x(r):
        return _layernorm(x_v[block_rows(r), :].astype(_F32)).astype(_BF16)

    def project_k(r, xn):
        k = jnp.dot(xn, wqkv_v[:, D:2 * D], preferred_element_type=_F32)
        for g in range(D // 128):
            kg = _pack(k[:, g * 128:(g + 1) * 128])
            rows = _aligned(r * (_QB // 2), _QB // 2)
            for j in range(HPG):
                k_v[g * HPG + j, rows, :] = pltpu.roll(kg, 128 - j * DH, 1) if j else kg

    def project_q(r):
        q = jnp.dot(_unpack(xn_v[...]), wqkv_v[:, 0:D], preferred_element_type=_F32)
        qt_v[r] = _pack((q * qscale).astype(_BF16).T)

    def project_v(r):
        v = jnp.dot(_unpack(xn_v[...]), wqkv_v[:, 2 * D:3 * D], preferred_element_type=_F32)
        vt_v[r] = _pack(v.astype(_BF16).T)

    def wqkv_copy(i):
        cols = pl.ds(i * D, D)
        return pltpu.make_async_copy(wqkv_hbm.at[:, cols], wqkv_v.at[:, cols], q_sem.at[i])

    x_copy(0).start()
    spare_s[0] = DH
    spare_s[1] = D
    spare_s[2] = F
    wqkv_copy(1).start()
    x_copy(0).wait()
    wqkv_copy(0).start()
    wqkv_copy(2).start()
    x_copy(1).start()
    xn_v[...] = _pack(norm_x(0))
    wqkv_copy(1).wait()
    project_k(0, _unpack(xn_v[...]))
    wqkv_copy(0).wait()
    wqkv_copy(2).wait()
    for r in range(2, NQ):
        x_copy(r).start()

    def combine_weights(qb, c, pace):
        if pace is not None:
            wgu_v[0, _aligned(spare_s[1], 16), 0:128] = pace[0:16].astype(_BF16)
            wd_v[_aligned(spare_s[2], 16), 0:128] = pace[64:80].astype(_BF16)
        gr, dr = D // 2 // NQ, 128 // NQ
        for j in range(c * (F // 128) // NC, (c + 1) * (F // 128) // NC):
            cols = pl.ds(j * 128, 128)
            top, bot = _aligned(qb * gr, gr), _aligned(qb * gr + D // 2, gr)
            blocks = (wgu_v[0, top, cols], wgu_v[1, top, cols],
                      wgu_v[0, bot, cols], wgu_v[1, bot, cols])
            for i, t in enumerate(_rhs5(*(b.astype(_F32) for b in blocks))):
                w5_v[i, _aligned(qb * (gr // 2), gr // 2), cols] = _pack(t)
            lo, hi = pl.ds(j % 2 * D // 4, D // 4), pl.ds((2 + j % 2) * D // 4, D // 4)
            top = _aligned(j // 2 * 256 + qb * dr, dr)
            bot = _aligned(j // 2 * 256 + 128 + qb * dr, dr)
            blocks = (wd_v[top, lo], wd_v[top, hi], wd_v[bot, lo], wd_v[bot, hi])
            for i, t in enumerate(_rhs5(*(b.astype(_F32) for b in blocks))):
                d5_v[i, _aligned(j // 2 * 64 + qb * (dr // 2), dr // 2), lo] = _pack(t)

    def qkv_block(r, _):
        x_copy(r + 1).wait()

        @pl.when(r == min(1, NQ - 2))
        def _():
            for cp in w_copies:
                cp.start()

        xn = norm_x(r + 1)
        project_q(r)
        project_k(r + 1, xn)
        project_v(r)
        xn_v[...] = _pack(xn)

    lax.fori_loop(0, NQ - 1, qkv_block, None)

    parts = [(g, t, ds) for g in range(len(_CK)) for t in range(_QB // _PQ)
             for ds in range(_DS)]
    parts_at = {}
    for j, (g, t, ds) in enumerate(parts):
        c = max(j * _C1 // len(parts), _CK[g] if ds == _DS - 1 else 0)
        parts_at.setdefault(c, []).append((g, t, ds))

    def head_rows(h):
        return _aligned(h * DH, DH)

    def load_q(qb, h):
        return _unpack(qt_v[qb, _aligned(h * (DH // 2), DH // 2), :])

    def load_k(h, row, nrows):
        return _unpack(k_v[h, pl.ds(row // 2, nrows // 2), :])

    def spread_k(h, g):
        k = load_k(h, _CK[g] * _KC, _PK).astype(_F32)
        for d in range(DH):
            kb_v[d, pl.ds(g * _PK, _PK), :] = jnp.broadcast_to(k[:, d:d + 1], (_PK, 128))

    def spread_q(qb, d, q):
        qb_v[qb, d] = jnp.broadcast_to(q[d:d + 1], (8, _QB))

    def softmax_pv(h, qb, c, m, acc, l):
        s = s_v[qb, pl.ds(c * _KC, _KC), :].reshape(_KC // 8, 8, _QB)
        p = jnp.exp2(s - m[None])
        for t in reversed(range(0, _KC // 8, 2)):
            l = _add(l, p[t] + p[t + 1])
        vt = _unpack(vt_v[c * _KC // _QB, _aligned(h * (DH // 2), DH // 2),
                          pl.ds(c * _KC % _QB, _KC)])
        return _add(acc, jnp.dot(vt, p.reshape(_KC, _QB).astype(_BF16),
                                 preferred_element_type=_F32)), l

    def store_o(h, qb, acc, l):
        o = acc / jnp.sum(l, axis=0, keepdims=True)
        for j in range(_QB // _RB):
            ot_v[qb * (_QB // _RB) + j, head_rows(h), :] = (
                o[:, j * _RB:(j + 1) * _RB].astype(_BF16))

    def scores(h, qb, q, row, nrows):
        s = jnp.dot(load_k(h, row, nrows)[:, 0:DH], q, preferred_element_type=_F32)
        s_v[qb, pl.ds(row, nrows), :] = s
        return s, jnp.max(s.reshape(nrows // 8, 8, _QB), axis=0)

    def row_max(m):
        return jnp.broadcast_to(jnp.max(m, axis=0, keepdims=True), (8, _QB))

    def first_scores(qb):
        q = load_q(qb, 0)
        m = jnp.full((8, _QB), -jnp.inf, _F32)
        pace = None
        for c in range(NC):
            combine_weights(qb, c, pace)
            s, top = scores(0, qb, q, c * _KC, _KC)
            pace = s[:, 0:128]
            m = jnp.maximum(m, top)
        return row_max(m)

    def attn_head(h, m_prev):
        spare = spare_s[0]
        pace = None
        h_next = jnp.minimum(h + 1, _H - 1)
        m_new = []
        for qb in range(NQ):
            q = load_q(qb, h)
            qb_next = (qb + 1) % NQ
            q_next = load_q(qb_next, h if qb_next else h_next).astype(_F32)
            partial = {}
            m = [jnp.full((8, _PQ), -jnp.inf, _F32)] * (_QB // _PQ)
            acc = l = None
            for c in range(NC):
                for d in range(c * DH // NC, (c + 1) * DH // NC):
                    spread_q(qb_next, d, q_next)
                acc, l = softmax_pv(h - 1, qb, c, m_prev[qb], acc, l)
                if pace is not None and c in parts_at:
                    kb_v[spare, 0:8, :] = pace
                for g, t, ds in parts_at.get(c, ()):
                    a = partial.get((g, t))
                    for d in range(ds * DH // _DS, (ds + 1) * DH // _DS):
                        k = kb_v[d, pl.ds(g * _PK, _PK), :].reshape(_PK // 8, 8, 128)
                        prod = (jnp.concatenate([k] * (_PQ // 128), axis=2)
                                * qb_v[qb, d, :, pl.ds(t * _PQ, _PQ)][None])
                        a = _add(a, prod)
                    partial[g, t] = a
                    if ds == _DS - 1:
                        s_v[qb, pl.ds(_CK[g] * _KC, _PK), pl.ds(t * _PQ, _PQ)] = (
                            a.reshape(_PK, _PQ))
                        m[t] = jnp.maximum(m[t], jnp.max(a, axis=0))
                        if qb == NQ - 1 and t == _QB // _PQ - 1:
                            spread_k(h_next, g)
                row = c * _KC + (_PK if c in _CK else 0)
                s, top = scores(h, qb, q, row, (c + 1) * _KC - row)
                pace = s[_TK * 8:_TK * 8 + 8, 0:128]
                m = [jnp.maximum(m[t], top[:, t * _PQ:(t + 1) * _PQ])
                     for t in range(_QB // _PQ)]
            store_o(h - 1, qb, acc, l)
            m_new.append(row_max(jnp.concatenate(m, axis=1)))
        return tuple(m_new)

    for cp in w_copies:
        cp.wait()
    project_q(NQ - 1)
    for g in range(len(_CK)):
        spread_k(1, g)
    for d in range(DH):
        spread_q(0, d, load_q(0, 1).astype(_F32))
    project_v(NQ - 1)
    ms = tuple(first_scores(qb) for qb in range(NQ))
    ms = lax.fori_loop(1, _H, attn_head, ms)

    early = [(t, kt) for t in range(_QB // 128) for kt in range(D // 128 - 1)]

    def last_pv(qb):
        acc = l = None
        for c in range(NC):
            acc, l = softmax_pv(_H - 1, qb, c, ms[qb], acc, l)
            for t, kt in early[c * len(early) // NC:(c + 1) * len(early) // NC]:
                j, lanes = divmod(t * 128, _RB)
                rows, depth = _aligned(qb * _QB + t * 128, 128), pl.ds(kt * 128, 128)
                part = lax.dot_general(
                    ot_v[qb * (_QB // _RB) + j, depth, pl.ds(lanes, 128)], wo_v[depth, :],
                    _TN, preferred_element_type=_F32)
                base = part + (x_v[rows, :].astype(_F32) if kt == 0 else base)
                if kt == D // 128 - 2:
                    hp_v[rows, :] = base
        store_o(_H - 1, qb, acc, l)

    NR = S // _RB

    R, DK = _RB // 2, D // 2

    def finish_h(r):
        depth = pl.ds(D - 128, 128)
        h = hp_v[_aligned(r * _RB, _RB), :] + lax.dot_general(
            ot_v[r, depth, :], wo_v[depth, :], _TN, preferred_element_type=_F32)
        h_v[r] = h
        n = _layernorm(h)
        for i, t in enumerate(_lhs7(n[:R, :DK], n[:R, DK:], n[R:, :DK], n[R:, DK:])):
            hx_v[i] = _pack(t)

    def swiglu(gate, up):
        half = 0.5 * gate
        return (half * up) * (1.0 + jnp.tanh(half))

    for qb in range(NQ):
        last_pv(qb)
        if qb == 1:
            finish_h(0)

    def ffn_block(r, _):
        hn_v[...] = hx_v[...]
        for j in range(F // 256):
            if j == _FJ:
                finish_h(jnp.minimum(r + 1, NR - 1))
            cols = pl.ds(j * 256, 256)
            w = _rhs7([_unpack(w5_v[i, :, cols]) for i in range(5)],
                      wgu_v[0, 0:DK, cols], wgu_v[1, DK:D, cols])
            g1, u1, g2, u2 = _out4([
                jnp.dot(_unpack(hn_v[i]), w[i], preferred_element_type=_F32)
                for i in range(7)])
            a1, a2 = swiglu(g1, u1), swiglu(g2, u2)
            for i, t in enumerate(_lhs7(a1[:, :128], a1[:, 128:], a2[:, :128], a2[:, 128:])):
                a_v[i, :, pl.ds(j * 128, 128)] = _pack(t)
        w = _rhs7([_unpack(d5_v[i]) for i in range(5)],
                  jnp.concatenate([wd_v[j:j + 128, 0:DK] for j in range(0, F, 256)], axis=0),
                  jnp.concatenate([wd_v[j:j + 128, DK:D] for j in range(128, F, 256)], axis=0))
        y11, y12, y21, y22 = _out4([
            jnp.dot(_unpack(a_v[i]), w[i], preferred_element_type=_F32) for i in range(7)])
        y = h_v[r] + jnp.concatenate([jnp.concatenate([y11, y12], axis=1),
                                        jnp.concatenate([y21, y22], axis=1)], axis=0)
        out_v[r] = y.astype(out_v.dtype)
        out_copy(r).start()

    lax.fori_loop(0, NR, ffn_block, None)
    for r in range(NR):
        out_copy(r).wait()


@jax.jit
def pallas_sequential_preLN__softmax_full_mha__swiglu_ffn__prompt_kernel(
    A_x: jax.Array,
    A_wqkv: jax.Array,
    A_wo: jax.Array,
    B_x: jax.Array,
    B_w_gate: jax.Array,
    B_w_up: jax.Array,
    B_w_down: jax.Array,
):
    del B_x
    B, S, D = A_x.shape
    F = B_w_gate.shape[1]
    assert B == 1 and S % _QB == 0 and D % 128 == 0 and F % 256 == 0
    assert S > _CK[-1] * _KC and _FJ < F // 256
    NQ = S // _QB
    any_spec = pl.BlockSpec(memory_space=pl.ANY)
    out = pl.pallas_call(
        functools.partial(_block_kernel, S=S, D=D, F=F),
        out_shape=jax.ShapeDtypeStruct((S, D), A_x.dtype),
        in_specs=[any_spec] * 6,
        out_specs=any_spec,
        scratch_shapes=[
            pltpu.VMEM((S, D), A_x.dtype),
            pltpu.VMEM((D, 3 * D), _BF16),
            pltpu.VMEM((D, D), _BF16),
            pltpu.VMEM((2, D + 16, F), _BF16),
            pltpu.VMEM((F + 16, D), _BF16),
            pltpu.VMEM((_H, S // 2, 128), jnp.uint32),
            pltpu.VMEM((NQ, D // 2, _QB), jnp.uint32),
            pltpu.VMEM((NQ, D // 2, _QB), jnp.uint32),
            pltpu.VMEM((S // _RB, D, _RB), _BF16),
            pltpu.VMEM((NQ, S, _QB), _F32),
            pltpu.VMEM((NQ, D // _H, 8, _QB), _F32),
            pltpu.VMEM((D // _H + 1, (len(_CK) + 1) * _PK, 128), _F32),
            pltpu.VMEM((_QB // 2, D), jnp.uint32),
            pltpu.VMEM((S, D), _F32),
            pltpu.VMEM((S // _RB, _RB, D), _F32),
            pltpu.VMEM((7, _RB // 4, D // 2), jnp.uint32),
            pltpu.VMEM((7, _RB // 4, D // 2), jnp.uint32),
            pltpu.VMEM((7, _RB // 4, F // 2), jnp.uint32),
            pltpu.VMEM((5, D // 4, F), jnp.uint32),
            pltpu.VMEM((5, F // 4, D // 2), jnp.uint32),
            pltpu.VMEM((S // _RB, _RB, D), A_x.dtype),
            pltpu.SMEM((3,), jnp.int32),
            pltpu.SemaphoreType.DMA((NQ,)),
            pltpu.SemaphoreType.DMA((3,)),
            pltpu.SemaphoreType.DMA((4,)),
            pltpu.SemaphoreType.DMA((S // _RB,)),
        ],
        compiler_params=pltpu.CompilerParams(
            vmem_limit_bytes=100 << 20,
            flags={"XLA_TPU_EVENLY_DISTRIBUTE_CRITICAL_NODES": True}),
    )(A_x.reshape(S, D), A_wqkv.astype(_BF16), A_wo.astype(_BF16),
      B_w_gate.astype(_BF16), B_w_up.astype(_BF16), B_w_down.astype(_BF16))
    return out.reshape(B, S, D)
```
